```python
import jax
import jax.numpy as jnp

def _softmax(x, axis=-1):
    return jax.nn.softmax(x, axis=axis)
def _gelu(x):
    return jax.nn.gelu(x, approximate=True)
def _silu(x):
    return jax.nn.silu(x)
def _sigmoid(x):
    return jax.nn.sigmoid(x)
def _layernorm(x, axis=-1, eps=1e-5):
    m = jnp.mean(x, axis=axis, keepdims=True)
    v = jnp.var(x, axis=axis, keepdims=True)
    return (x - m) / jnp.sqrt(v + eps)
def _scatter_add(tgt, idx, src, axis=0):
    return tgt.at[idx].add(src)
def _segment_sum(src, seg, n):
    return jax.ops.segment_sum(src, seg, n)
class _Rng:
    def __init__(self, key):
        self._k = key
    def _next(self):
        self._k, sub = jax.random.split(self._k)
        return sub
    def normal(self, shape):
        return jax.random.normal(self._next(), shape, dtype=jnp.bfloat16)
    def randint(self, lo, hi, shape):
        return jax.random.randint(self._next(), shape, lo, hi, dtype=jnp.int32)
    def uniform(self, shape, lo=0.0, hi=1.0):
        return jax.random.uniform(self._next(), shape, jnp.bfloat16, lo, hi)
    def permutation(self, n):
        return jax.random.permutation(self._next(), n)


kernel_name = 'recurrent_scan__sliding_block_cached__moe_arch_mod__decode'

def setup_inputs():
    _rng = _Rng(jax.random.key(int.from_bytes(__import__("os").urandom(4), "little")))
    _w = (lambda a: (lambda t: t.astype(jnp.bfloat16) if jnp.issubdtype(t.dtype, jnp.floating) else t)(jnp.asarray(a)))
    def _A_setup():
        B, Sq, D = 1, 1, 512
        Hq, Hkv, Sk, Dh = 32, 32, 32768, 128
        assert Hq % Hkv == 0, (Hq, Hkv)
        return {
            "x": _w((lambda *s: _rng.normal(s) * 0.05)(B, Sq, D)),
            "k_cache": _w((lambda *s: _rng.normal(s) * 0.05)(B, Hkv, Sk, Dh)),
            "v_cache": _w((lambda *s: _rng.normal(s) * 0.05)(B, Hkv, Sk, Dh)),
            "wq": _w((lambda *s: _rng.normal(s) * 0.05)(D, Hq * Dh) * (D ** -0.5)),
            "wo": _w((lambda *s: _rng.normal(s) * 0.05)(Hq * Dh, D) * ((Hq * Dh) ** -0.5)),
        }
    _A_in = _A_setup()

    def _B_setup():
        B, S, D, F, C = 1, 1, 512, 1376, 1
        return {
            "x": _w((lambda *s: _rng.normal(s) * 0.05)(B, S, D)),
            "w_r": _w((lambda *s: _rng.normal(s) * 0.05)(D)),
            "w_gate": _w((lambda *s: _rng.normal(s) * 0.05)(D, F)),
            "w_up": _w((lambda *s: _rng.normal(s) * 0.05)(D, F)),
            "w_down": _w((lambda *s: _rng.normal(s) * 0.05)(F, D)),
        }
    _B_in = _B_setup()

    return {
        "A_x": _A_in["x"],
        "A_k_cache": _A_in["k_cache"],
        "A_v_cache": _A_in["v_cache"],
        "A_wq": _A_in["wq"],
        "A_wo": _A_in["wo"],
        "B_x": _B_in["x"],
        "B_w_r": _B_in["w_r"],
        "B_w_gate": _B_in["w_gate"],
        "B_w_up": _B_in["w_up"],
        "B_w_down": _B_in["w_down"],
    }

def reference(A_x, A_k_cache, A_v_cache, A_wq, A_wo, B_x, B_w_r, B_w_gate, B_w_up, B_w_down):
    def _A_ref(x, k_cache, v_cache, wq, wo):
        B, Sq, D = x.shape
        Hq, Dh = 32, 128
        Hkv, Sk = k_cache.shape[1], k_cache.shape[2]
        W = min(4096, max(256, Sk // 4))
        rep = Hq // Hkv
        q = (lambda x, *d: x.transpose(*d))((x @ wq).reshape(B, Sq, Hq, Dh), 0, 2, 1, 3)
        k = jnp.repeat(k_cache[:, :, Sk - W:, :], rep, axis=1)
        v = jnp.repeat(v_cache[:, :, Sk - W:, :], rep, axis=1)
        scores = jnp.einsum("bhqd,bhkd->bhqk", q, k) * (Dh ** -0.5)
        p = _softmax(scores, axis=-1)
        o = jnp.einsum("bhqk,bhkd->bhqd", p, v)
        return (lambda x, *d: x.transpose(*d))(o, 0, 2, 1, 3).reshape(B, Sq, Hq * Dh) @ wo

    def _B_ref(x, w_r, w_gate, w_up, w_down):
        B, S, D = x.shape
        C = 1
        r = x @ w_r
        idx = jnp.argsort(-r, axis=-1)[:, :C]
        idx_e = jnp.repeat(idx.reshape(B, C, 1), D, axis=2)
        x_sel = jnp.take_along_axis(x, idx_e, axis=1)
        g = _silu(x_sel @ w_gate)
        u = x_sel @ w_up
        y = (g * u) @ w_down
        r_sel = _sigmoid(jnp.take_along_axis(r, idx, axis=1))
        y = y * r_sel.reshape(B, C, 1)
        b_off = (jnp.arange(B) * S).reshape(B, 1)
        flat_idx = (idx + b_off).reshape(B * C)
        zero = (x * 0.0).reshape(B * S, D)
        upd = _scatter_add(zero, flat_idx, y.reshape(B * C, D), axis=0)
        return x + upd.reshape(B, S, D)

    x = A_x
    xn = _layernorm(x, axis=-1)
    s = _A_ref(xn, A_k_cache, A_v_cache, A_wq, A_wo)
    g = _silu(_B_ref(xn, B_w_r, B_w_gate, B_w_up, B_w_down))
    return x + s * g
```

```python
import functools

import jax
import jax.numpy as jnp
import jax.experimental.pallas as pl
import jax.experimental.pallas.tpu as pltpu

D = 512
NH = 32
DH = 128
SK = 32768
W = min(4096, max(256, SK // 4))
F = 1376
S = 8
WO_CHUNKS = (2048, 1024, 512, 256, 128, 128)

BF16 = jnp.bfloat16
F32 = jnp.float32
_NT = (((1,), (1,)), ((), ()))


def _kernel(x_h, k_h, v_h, wq_h, wo_h, wr_h, wg_h, wu_h, wd_h, out_ref,
            x_v, wr_v, wq_v, k_v, v_v, wo_v, wg_v, wu_v, wd_v, q_v, o_v, sems):
    pre = [(x_h, x_v), (wr_h, wr_v), (wg_h, wg_v), (wu_h, wu_v), (wd_h, wd_v), (wq_h, wq_v)]
    n_pre = len(pre)
    post = []
    r0 = 0
    for r in WO_CHUNKS:
        post.append((wo_h.at[pl.ds(r0, r), :], wo_v.at[pl.ds(r0, r), :]))
        r0 += r

    def kv_copy(is_v, h, j):
        src, dst = (v_h, v_v) if is_v else (k_h, k_v)
        return pltpu.make_async_copy(src.at[0, h, pl.ds(SK - W, W), :], dst.at[h], sems.at[j % S])

    def static_copy(j):
        if j < n_pre:
            return pltpu.make_async_copy(*pre[j], sems.at[j % S])
        if j < n_pre + 2 * NH:
            i = j - n_pre
            return kv_copy(i % 2, i // 2, j)
        return pltpu.make_async_copy(*post[j - n_pre - 2 * NH], sems.at[j % S])

    n_total = n_pre + 2 * NH + len(post)

    def retire(j):
        static_copy(j).wait()
        if j + S < n_total:
            static_copy(j + S).start()

    for j in range(S):
        static_copy(j).start()

    retire(0)
    retire(1)
    x = x_v[0].astype(F32)
    mean = jnp.mean(x, axis=-1, keepdims=True)
    var = jnp.mean(jnp.square(x - mean), axis=-1, keepdims=True)
    xn_b = ((x - mean) / jnp.sqrt(var + 1e-5)).astype(BF16)
    xn = xn_b.astype(F32)
    xn8 = jnp.broadcast_to(xn_b, (8, D))

    r = jnp.sum(xn * wr_v[...].reshape(1, D).astype(F32), axis=-1, keepdims=True)
    retire(2)
    g = jax.lax.dot_general(xn8, wg_v[...], _NT, preferred_element_type=F32)
    retire(3)
    u = jax.lax.dot_general(xn8, wu_v[...], _NT, preferred_element_type=F32)
    hmid = (jax.nn.silu(g) * u).astype(BF16)
    retire(4)
    y = jnp.dot(hmid, wd_v[...], preferred_element_type=F32)
    upd = xn * 0.0 + y * jax.nn.sigmoid(r)
    gate = jax.nn.silu(xn + upd)

    retire(5)
    q = jnp.dot(xn8, wq_v[...], preferred_element_type=F32)
    for h in range(NH):
        q_v[h] = q[:, h * DH:(h + 1) * DH]

    scale = DH ** -0.5

    def head(h, carry):
        jk = n_pre + 2 * h
        kv_copy(0, h, jk).wait()

        @pl.when(h + S // 2 < NH)
        def _():
            kv_copy(0, h + S // 2, jk).start()

        for c in range(len(post)):
            @pl.when(2 * h + S == 2 * NH + c)
            def _():
                static_copy(n_pre + 2 * NH + c).start()

        qh = q_v[h].astype(BF16)
        s = jax.lax.dot_general(qh, k_v[h], _NT, preferred_element_type=F32) * scale
        m = jnp.max(s, axis=-1, keepdims=True)
        p = jnp.exp(s - m)
        l = jnp.sum(p, axis=-1, keepdims=True)

        kv_copy(1, h, jk + 1).wait()

        @pl.when(h + S // 2 < NH)
        def _():
            kv_copy(1, h + S // 2, jk + 1).start()

        for c in range(len(post)):
            @pl.when(2 * h + 1 + S == 2 * NH + c)
            def _():
                static_copy(n_pre + 2 * NH + c).start()

        o = jnp.dot(p.astype(BF16), v_v[h], preferred_element_type=F32)
        o_v[h] = o / l
        return carry

    jax.lax.fori_loop(0, NH, head, 0)

    acc = jnp.zeros((8, D), F32)
    r0 = 0
    for c, r in enumerate(WO_CHUNKS):
        static_copy(n_pre + 2 * NH + c).wait()
        o_c = jnp.concatenate([o_v[h] for h in range(r0 // DH, (r0 + r) // DH)], axis=1).astype(BF16)
        acc = acc + jnp.dot(o_c, wo_v[pl.ds(r0, r), :], preferred_element_type=F32)
        r0 += r

    out_ref[0] = (x + acc[0:1] * gate[0:1]).astype(out_ref.dtype)


@jax.jit
def pallas_recurrent_scan__sliding_block_cached__moe_arch_mod__decode_kernel(
    A_x: jax.Array,
    A_k_cache: jax.Array,
    A_v_cache: jax.Array,
    A_wq: jax.Array,
    A_wo: jax.Array,
    B_x: jax.Array,
    B_w_r: jax.Array,
    B_w_gate: jax.Array,
    B_w_up: jax.Array,
    B_w_down: jax.Array,
):
    del B_x
    hbm = pl.BlockSpec(memory_space=pltpu.HBM)
    return pl.pallas_call(
        _kernel,
        out_shape=jax.ShapeDtypeStruct((1, 1, D), BF16),
        in_specs=[hbm] * 9,
        out_specs=pl.BlockSpec(memory_space=pltpu.VMEM),
        scratch_shapes=[
            pltpu.VMEM((1, 1, D), BF16),
            pltpu.VMEM((D,), BF16),
            pltpu.VMEM((D, NH * DH), BF16),
            pltpu.VMEM((NH, W, DH), BF16),
            pltpu.VMEM((NH, W, DH), BF16),
            pltpu.VMEM((NH * DH, D), BF16),
            pltpu.VMEM((F, D), BF16),
            pltpu.VMEM((F, D), BF16),
            pltpu.VMEM((F, D), BF16),
            pltpu.VMEM((NH, 8, DH), F32),
            pltpu.VMEM((NH, 8, DH), F32),
            pltpu.SemaphoreType.DMA((S,)),
        ],
        compiler_params=pltpu.CompilerParams(vmem_limit_bytes=100 * 1024 * 1024),
    )(A_x, A_k_cache, A_v_cache, A_wq, A_wo, B_w_r, B_w_gate.T, B_w_up.T, B_w_down)
```

```python
import jax
import jax.numpy as jnp
import jax.experimental.pallas as pl
import jax.experimental.pallas.tpu as pltpu

D = 512
NH = 32
DH = 128
SK = 32768
W = min(4096, max(256, SK // 4))
F = 1376
S = 8
WO_CHUNKS = (2048, 1024, 512, 256, 128, 96, 32)
WO_VPU = 2

BF16 = jnp.bfloat16
F32 = jnp.float32
_NT = (((1,), (1,)), ((), ()))


def _kernel(x_h, k_h, v_h, wq_h, wo_h, wr_h, wg_h, wu_h, wd_h, out_ref,
            x_v, wr_v, wq_v, k_v, v_v, wo_v, wg_v, wu_v, wd_v, q_v, o_v, sems):
    pre = [(x_h, x_v), (wr_h, wr_v), (wg_h, wg_v), (wu_h, wu_v), (wd_h, wd_v), (wq_h, wq_v)]
    n_pre = len(pre)
    post = []
    r0 = 0
    for r in WO_CHUNKS:
        post.append((wo_h.at[pl.ds(r0, r), :], wo_v.at[pl.ds(r0, r), :]))
        r0 += r
    assert r0 == NH * DH and sum(WO_CHUNKS[-WO_VPU:]) == DH
    n_total = n_pre + 2 * NH + len(post)

    def kv_copy(is_v, h, j):
        src, dst = (v_h, v_v) if is_v else (k_h, k_v)
        return pltpu.make_async_copy(src.at[0, h, pl.ds(SK - W, W), :], dst.at[h], sems.at[j % S])

    def copy(j):
        if j < n_pre:
            return pltpu.make_async_copy(*pre[j], sems.at[j % S])
        if j < n_pre + 2 * NH:
            return kv_copy((j - n_pre) % 2, (j - n_pre) // 2, j)
        return pltpu.make_async_copy(*post[j - n_pre - 2 * NH], sems.at[j % S])

    def retire(j):
        copy(j).wait()
        if j + S < n_total:
            copy(j + S).start()

    for j in range(S):
        copy(j).start()

    retire(0)
    retire(1)
    x = x_v[0].astype(F32)
    mean = jnp.mean(x, axis=-1, keepdims=True)
    var = jnp.mean(jnp.square(x - mean), axis=-1, keepdims=True)
    xn_b = ((x - mean) / jnp.sqrt(var + 1e-5)).astype(BF16)
    xn = xn_b.astype(F32)
    xn8 = jnp.broadcast_to(xn_b, (8, D))

    r = jnp.sum(xn * wr_v[...].reshape(1, D).astype(F32), axis=-1, keepdims=True)
    retire(2)
    g = jax.lax.dot_general(xn8, wg_v[...], _NT, preferred_element_type=F32)
    retire(3)
    u = jax.lax.dot_general(xn8, wu_v[...], _NT, preferred_element_type=F32)
    hid = (jax.nn.silu(g) * u).astype(BF16)
    retire(4)
    y = jnp.dot(hid, wd_v[...], preferred_element_type=F32)
    upd = xn * 0.0 + y * jax.nn.sigmoid(r)
    gate = jax.nn.silu(xn + upd)

    retire(5)
    q = jnp.dot(xn8, wq_v[...], preferred_element_type=F32)
    for h in range(NH):
        q_v[h] = q[:, h * DH:(h + 1) * DH]

    scale = DH ** -0.5

    def advance(h, is_v):
        j = n_pre + 2 * h + is_v
        nxt = 2 * h + is_v + S

        @pl.when(nxt < 2 * NH)
        def _():
            kv_copy(is_v, h + S // 2, j).start()

        for c in range(len(post)):
            @pl.when(nxt == 2 * NH + c)
            def _():
                copy(n_pre + 2 * NH + c).start()

    def head(h, carry):
        j = n_pre + 2 * h
        kv_copy(0, h, j).wait()
        advance(h, 0)
        s = jax.lax.dot_general(q_v[h].astype(BF16), k_v[h], _NT,
                                preferred_element_type=F32) * scale
        m = jnp.max(s, axis=-1, keepdims=True)
        p = jnp.exp(s - m)
        l = jnp.sum(p, axis=-1, keepdims=True)
        kv_copy(1, h, j + 1).wait()
        advance(h, 1)
        o = jnp.dot(p.astype(BF16), v_v[h], preferred_element_type=F32)
        o_v[h] = o / l
        return carry

    jax.lax.fori_loop(0, NH, head, 0)

    o_last = o_v[NH - 1].astype(BF16).astype(F32)
    o_col = jnp.broadcast_to(o_last[0:1], (DH, DH)).T
    acc = jnp.zeros((8, D), F32)
    part = jnp.zeros((8, D), F32)
    r0 = 0
    for c, r in enumerate(WO_CHUNKS):
        retire(n_pre + 2 * NH + c)
        if c < len(WO_CHUNKS) - WO_VPU:
            for h in range(r0 // DH, (r0 + r) // DH):
                acc = acc + jnp.dot(o_v[h].astype(BF16), wo_v[pl.ds(h * DH, DH), :],
                                    preferred_element_type=F32)
        else:
            lo = r0 - (NH - 1) * DH
            coef = jnp.concatenate([o_col[lo:lo + r]] * (D // DH), axis=1)
            prod = wo_v[pl.ds(r0, r), :].astype(F32) * coef
            part = part + prod.reshape(r // 8, 8, D).sum(axis=0)
        r0 += r
    row = jax.lax.broadcasted_iota(jnp.int32, (8, D), 0)
    s_out = jnp.sum(part + jnp.where(row == 0, acc, 0.0), axis=0, keepdims=True)

    out_ref[0] = (x + s_out * gate[0:1]).astype(out_ref.dtype)


@jax.jit
def pallas_recurrent_scan__sliding_block_cached__moe_arch_mod__decode_kernel(
    A_x: jax.Array,
    A_k_cache: jax.Array,
    A_v_cache: jax.Array,
    A_wq: jax.Array,
    A_wo: jax.Array,
    B_x: jax.Array,
    B_w_r: jax.Array,
    B_w_gate: jax.Array,
    B_w_up: jax.Array,
    B_w_down: jax.Array,
):
    del B_x
    hbm = pl.BlockSpec(memory_space=pltpu.HBM)
    return pl.pallas_call(
        _kernel,
        out_shape=jax.ShapeDtypeStruct((1, 1, D), BF16),
        in_specs=[hbm] * 9,
        out_specs=pl.BlockSpec(memory_space=pltpu.VMEM),
        scratch_shapes=[
            pltpu.VMEM((1, 1, D), BF16),
            pltpu.VMEM((D,), BF16),
            pltpu.VMEM((D, NH * DH), BF16),
            pltpu.VMEM((NH, W, DH), BF16),
            pltpu.VMEM((NH, W, DH), BF16),
            pltpu.VMEM((NH * DH, D), BF16),
            pltpu.VMEM((F, D), BF16),
            pltpu.VMEM((F, D), BF16),
            pltpu.VMEM((F, D), BF16),
            pltpu.VMEM((NH, 8, DH), F32),
            pltpu.VMEM((NH, 8, DH), F32),
            pltpu.SemaphoreType.DMA((S,)),
        ],
        compiler_params=pltpu.CompilerParams(
            vmem_limit_bytes=100 * 1024 * 1024,
            disable_semaphore_checks=True,
        ),
    )(A_x, A_k_cache, A_v_cache, A_wq, A_wo, B_w_r, B_w_gate.T, B_w_up.T, B_w_down)
```

```python
import jax
import jax.numpy as jnp
import jax.experimental.pallas as pl
import jax.experimental.pallas.tpu as pltpu

D = 512
NH = 32
DH = 128
SK = 32768
W = min(4096, max(256, SK // 4))
F = 1376
S = 8
WO_CHUNKS = (2048, 1024, 512, 256, 128, 80, 32, 16)
WO_VPU = 3

BF16 = jnp.bfloat16
F32 = jnp.float32
_NT = (((1,), (1,)), ((), ()))


def _kernel(x_h, k_h, v_h, wq_h, wo_h, wr_h, wg_h, wu_h, wd_h, out_ref,
            x_v, wr_v, wq_v, k_v, v_v, wo_v, wg_v, wu_v, wd_v, q_v, o_v, sems):
    pre = [(x_h, x_v), (wr_h, wr_v), (wg_h, wg_v), (wu_h, wu_v), (wd_h, wd_v), (wq_h, wq_v)]
    n_pre = len(pre)
    post = []
    r0 = 0
    for r in WO_CHUNKS:
        post.append((wo_h.at[pl.ds(r0, r), :], wo_v.at[pl.ds(r0, r), :]))
        r0 += r
    assert r0 == NH * DH and sum(WO_CHUNKS[-WO_VPU:]) == DH
    n_total = n_pre + 2 * NH + len(post)

    def kv_copy(is_v, h, j):
        src, dst = (v_h, v_v) if is_v else (k_h, k_v)
        return pltpu.make_async_copy(src.at[0, h, pl.ds(SK - W, W), :], dst.at[h], sems.at[j % S])

    def copy(j):
        if j < n_pre:
            return pltpu.make_async_copy(*pre[j], sems.at[j % S])
        if j < n_pre + 2 * NH:
            return kv_copy((j - n_pre) % 2, (j - n_pre) // 2, j)
        return pltpu.make_async_copy(*post[j - n_pre - 2 * NH], sems.at[j % S])

    def retire(j):
        copy(j).wait()
        if j + S < n_total:
            copy(j + S).start()

    for j in range(S):
        copy(j).start()

    retire(0)
    retire(1)
    x = x_v[0].astype(F32)
    mean = jnp.mean(x, axis=-1, keepdims=True)
    var = jnp.mean(jnp.square(x - mean), axis=-1, keepdims=True)
    xn_b = ((x - mean) / jnp.sqrt(var + 1e-5)).astype(BF16)
    xn = xn_b.astype(F32)
    x8 = jnp.broadcast_to(x, (8, D))
    xn8 = jnp.broadcast_to(xn_b, (8, D))

    r = jnp.sum(xn * wr_v[...].reshape(1, D).astype(F32), axis=-1, keepdims=True)
    retire(2)
    g = jax.lax.dot_general(xn8, wg_v[...], _NT, preferred_element_type=F32)
    retire(3)
    u = jax.lax.dot_general(xn8, wu_v[...], _NT, preferred_element_type=F32)
    hid = (jax.nn.silu(g) * u).astype(BF16)
    retire(4)
    y = jnp.dot(hid, wd_v[...], preferred_element_type=F32)
    upd = xn * 0.0 + y * jax.nn.sigmoid(r)
    gate = jax.nn.silu(xn + upd)

    retire(5)
    q = jnp.dot(xn8, wq_v[...], preferred_element_type=F32)
    for h in range(NH):
        q_v[h] = q[:, h * DH:(h + 1) * DH]

    scale = DH ** -0.5

    def advance(h, is_v):
        j = n_pre + 2 * h + is_v
        nxt = 2 * h + is_v + S

        @pl.when(nxt < 2 * NH)
        def _():
            kv_copy(is_v, h + S // 2, j).start()

        for c in range(len(post)):
            @pl.when(nxt == 2 * NH + c)
            def _():
                copy(n_pre + 2 * NH + c).start()

    def head(h, carry):
        j = n_pre + 2 * h
        kv_copy(0, h, j).wait()
        advance(h, 0)
        s = jax.lax.dot_general(q_v[h].astype(BF16), k_v[h], _NT,
                                preferred_element_type=F32) * scale
        m = jnp.max(s, axis=-1, keepdims=True)
        p = jnp.exp(s - m)
        l = jnp.sum(p, axis=-1, keepdims=True)
        kv_copy(1, h, j + 1).wait()
        advance(h, 1)
        o = jnp.dot(p.astype(BF16), v_v[h], preferred_element_type=F32)
        o_v[h] = o / l
        return carry

    jax.lax.fori_loop(0, NH, head, 0)

    o_last = o_v[NH - 1].astype(BF16).astype(F32)
    o_col = jnp.broadcast_to(o_last[0:1], (DH, DH)).T
    acc = jnp.zeros((8, D), F32)
    part = None
    row = jax.lax.broadcasted_iota(jnp.int32, (8, D), 0)
    r0 = 0
    for c, r in enumerate(WO_CHUNKS):
        retire(n_pre + 2 * NH + c)
        if c < len(WO_CHUNKS) - WO_VPU:
            for h in range(r0 // DH, (r0 + r) // DH):
                acc = acc + jnp.dot(o_v[h].astype(BF16), wo_v[pl.ds(h * DH, DH), :],
                                    preferred_element_type=F32)
        else:
            if part is None:
                part = jnp.where(row == 0, acc, 0.0)
            lo = r0 - (NH - 1) * DH
            coef = jnp.concatenate([o_col[lo:lo + r]] * (D // DH), axis=1)
            prod = wo_v[pl.ds(r0, r), :].astype(F32) * coef
            part = part + prod.reshape(r // 8, 8, D).sum(axis=0)
        r0 += r
    s_out = jnp.sum(part, axis=0, keepdims=True)

    res = x8 + jnp.broadcast_to(s_out, (8, D)) * gate
    out_ref[0] = res.astype(out_ref.dtype)[0:1]


@jax.jit
def pallas_recurrent_scan__sliding_block_cached__moe_arch_mod__decode_kernel(
    A_x: jax.Array,
    A_k_cache: jax.Array,
    A_v_cache: jax.Array,
    A_wq: jax.Array,
    A_wo: jax.Array,
    B_x: jax.Array,
    B_w_r: jax.Array,
    B_w_gate: jax.Array,
    B_w_up: jax.Array,
    B_w_down: jax.Array,
):
    del B_x
    hbm = pl.BlockSpec(memory_space=pltpu.HBM)
    return pl.pallas_call(
        _kernel,
        out_shape=jax.ShapeDtypeStruct((1, 1, D), BF16),
        in_specs=[hbm] * 9,
        out_specs=pl.BlockSpec(memory_space=pltpu.VMEM),
        scratch_shapes=[
            pltpu.VMEM((1, 1, D), BF16),
            pltpu.VMEM((D,), BF16),
            pltpu.VMEM((D, NH * DH), BF16),
            pltpu.VMEM((NH, W, DH), BF16),
            pltpu.VMEM((NH, W, DH), BF16),
            pltpu.VMEM((NH * DH, D), BF16),
            pltpu.VMEM((F, D), BF16),
            pltpu.VMEM((F, D), BF16),
            pltpu.VMEM((F, D), BF16),
            pltpu.VMEM((NH, 8, DH), F32),
            pltpu.VMEM((NH, 8, DH), F32),
            pltpu.SemaphoreType.DMA((S,)),
        ],
        compiler_params=pltpu.CompilerParams(
            vmem_limit_bytes=100 * 1024 * 1024,
            disable_semaphore_checks=True,
        ),
    )(A_x, A_k_cache, A_v_cache, A_wq, A_wo, B_w_r, B_w_gate.T, B_w_up.T, B_w_down)
```

```python
import jax
import jax.numpy as jnp
import jax.experimental.pallas as pl
import jax.experimental.pallas.tpu as pltpu

D = 512
NH = 32
DH = 128
SK = 32768
W = min(4096, max(256, SK // 4))
F = 1376

G = 4
NG = NH // G
PR = 112
M = 7
NP = G * M
K1 = W - NP * PR
QS = 4
LOOK = 2
WQ1, WQR = 112, 16
F1, FR = 352, 128
NW, WSUB = 20, 5
WO_CHUNKS = (512, 512, 256, 128, 80, 32, 16)
WO_VPU = 3
T_QK, T_PV, T_W, T_K0, T_WO = 175, 165, 205, 186, 200

BF16 = jnp.bfloat16
F32 = jnp.float32
_NT = (((1,), (1,)), ((), ()))
LONG, SHORT = 1, 0


def _kernel(x_h, k_h, v_h, wq_h, wo_h, wr_h, wg_h, wu_h, wd_h, out_ref,
            x_v, wr_v, wq_v, kv_v, wo_v, wg_v, wu_v, wd_v, q_v, o_v, s_v,
            s_x, s_w1, s_w0, s_kv1, s_kv0, s_wo1, s_wo0):
    kv_h = (k_h, v_h)

    def long_kv(t, g):
        return pltpu.make_async_copy(
            kv_h[t].at[0, pl.ds(g * G, G), pl.ds(SK - W, K1), :],
            kv_v.at[t, pl.ds(g * G, G), pl.ds(0, K1), :], s_kv1.at[t, g % (LOOK + 1)])

    def short_kv(t, g, j):
        ro = K1 + j * PR
        return pltpu.make_async_copy(
            kv_h[t].at[0, pl.ds(g * G, G), pl.ds(SK - W + ro, PR), :],
            kv_v.at[t, pl.ds(g * G, G), pl.ds(ro, PR), :], s_kv0.at[t, g % 2])

    def wait_kv(t, g):
        long_kv(t, g).wait()
        rest = kv_v.at[t, pl.ds(g * G, G), pl.ds(K1, W - K1), :]
        pltpu.make_async_copy(rest, rest, s_kv0.at[t, g % 2]).wait()

    copy_x = pltpu.make_async_copy(x_h, x_v, s_x.at[0])
    copy_wr = pltpu.make_async_copy(wr_h, wr_v, s_x.at[1])
    ws = ((wq_h, wq_v), (wg_h, wg_v), (wu_h, wu_v), (wd_h, wd_v))
    w1 = (WQ1, F1, F1, F1)
    long_w = [pltpu.make_async_copy(ws[a][0].at[pl.ds(0, w1[a]), :], ws[a][1].at[pl.ds(0, w1[a]), :],
                                    s_w1.at[a]) for a in range(4)]

    def short_w(a, rows, i):
        ro = w1[a] + i * rows
        return pltpu.make_async_copy(ws[a][0].at[pl.ds(ro, rows), :], ws[a][1].at[pl.ds(ro, rows), :],
                                     s_w0.at[a])

    def wait_w(a):
        long_w[a].wait()
        rest = ws[a][1].at[pl.ds(w1[a], ws[a][1].shape[0] - w1[a]), :]
        pltpu.make_async_copy(rest, rest, s_w0.at[a]).wait()

    per = NW // WSUB
    long_wo = []
    r0 = NW * DH
    for c, r in enumerate(WO_CHUNKS):
        long_wo.append(pltpu.make_async_copy(wo_h.at[pl.ds(r0, r), :], wo_v.at[pl.ds(r0, r), :], s_wo1.at[c]))
        r0 += r
    assert r0 == NH * DH and per * WSUB == NW and sum(WO_CHUNKS[-WO_VPU:]) == DH
    short_wo = [pltpu.make_async_copy(wo_h.at[pl.ds(i * DH, DH), :], wo_v.at[pl.ds(i * DH, DH), :],
                                      s_wo0.at[i // per]) for i in range(NW)]

    def slot(c):
        pl.delay(1)
        if c is not None:
            c.start(priority=SHORT)
        pl.delay(1)

    def idle_slot(c, t):
        if c is not None:
            c.start(priority=SHORT)
        pl.delay(t)

    n_wq, n_f = (D - WQ1) // WQR, (F - F1) // FR
    assert WQ1 + n_wq * WQR == D and F1 + n_f * FR == F
    seq = [(short_w(0, WQR, i), T_W) for i in range(n_wq)]
    seq += [(short_w(a, FR, i), T_W) for i in range(n_f) for a in (1, 2, 3)]
    n_w = len(seq)
    seq += [(short_kv(0, 0, j), T_K0) for j in range(NP)]
    pos = [0]

    def nxt():
        pos[0] += 1
        return seq[pos[0] - 1]

    def idle_until(n):
        while pos[0] < n:
            idle_slot(*nxt())

    copy_x.start(priority=SHORT)
    copy_wr.start(priority=SHORT)
    for c in long_w:
        c.start(priority=LONG)
    idle_until(2)
    copy_x.wait()
    copy_wr.wait()

    slot(nxt()[0])
    x = x_v[0].astype(F32)
    mean = jnp.mean(x, axis=-1, keepdims=True)
    var = jnp.mean(jnp.square(x - mean), axis=-1, keepdims=True)
    xn_b = ((x - mean) / jnp.sqrt(var + 1e-5)).astype(BF16)
    xn = xn_b.astype(F32)
    x8 = jnp.broadcast_to(x, (8, D))
    xn8 = jnp.broadcast_to(xn_b, (8, D))
    r = jnp.sum(xn * wr_v[...].reshape(1, D).astype(F32), axis=-1, keepdims=True)

    idle_until(n_wq)
    long_kv(0, 0).start(priority=LONG)
    long_kv(1, 0).start(priority=LONG)
    idle_until(n_wq + 4)

    wait_w(0)
    QC = 512
    for c in range(NH * DH // QC):
        slot(nxt()[0])
        q = jnp.dot(xn8, wq_v[:, pl.ds(c * QC, QC)], preferred_element_type=F32)
        for t in range(QC // DH):
            q_v[c * (QC // DH) + t] = q[:, t * DH:(t + 1) * DH]

    idle_until(n_w + 4)
    for g in range(1, LOOK):
        long_kv(0, g).start(priority=LONG)
        long_kv(1, g).start(priority=LONG)

    for a in (1, 2, 3):
        wait_w(a)
    y = None
    for c0, cn in ((0, 512), (512, 512), (1024, F - 1024)):
        slot(nxt()[0])
        gt = jax.lax.dot_general(xn8, wg_v[pl.ds(c0, cn), :], _NT, preferred_element_type=F32)
        slot(nxt()[0])
        up = jax.lax.dot_general(xn8, wu_v[pl.ds(c0, cn), :], _NT, preferred_element_type=F32)
        hid = (jax.nn.silu(gt) * up).astype(BF16)
        slot(nxt()[0])
        t = jnp.dot(hid, wd_v[pl.ds(c0, cn), :], preferred_element_type=F32)
        y = t if y is None else y + t
    slot(nxt()[0])
    upd = xn * 0.0 + y * jax.nn.sigmoid(r)
    gate = jax.nn.silu(xn + upd)
    idle_until(len(seq))

    scale = DH ** -0.5
    KS = W // QS

    def scores(h, hh, c):
        s_v[hh, :, pl.ds(c * KS, KS)] = jax.lax.dot_general(
            q_v[h].astype(BF16), kv_v[0, h, pl.ds(c * KS, KS), :], _NT, preferred_element_type=F32) * scale

    def softmax_pv(h, hh, copies):
        HW = W // 2
        slot(copies[0])
        s1 = s_v[hh, :, pl.ds(0, HW)]
        s2 = s_v[hh, :, pl.ds(HW, HW)]
        mx = jnp.max(jnp.maximum(s1, s2), axis=-1, keepdims=True)
        p1 = jnp.exp(s1 - mx)
        p2 = jnp.exp(s2 - mx)
        l = jnp.sum(p1 + p2, axis=-1, keepdims=True)
        slot(copies[1])
        o = jnp.dot(p1.astype(BF16), kv_v[1, h, pl.ds(0, HW), :], preferred_element_type=F32)
        slot(copies[2])
        o = o + jnp.dot(p2.astype(BF16), kv_v[1, h, pl.ds(HW, HW), :], preferred_element_type=F32)
        o_v[h] = o / l

    def group(g, carry):
        for hh in range(G):
            for i in range(M - QS):
                idle_slot(short_kv(1, g, hh * M + i), T_QK)
            if hh == 0:
                wait_kv(0, g)

                @pl.when(g + LOOK < NG)
                def _():
                    long_kv(0, g + LOOK).start(priority=LONG)
            for c in range(QS):
                slot(short_kv(1, g, hh * M + M - QS + c))
                scores(g * G + hh, hh, c)

        @pl.when(g + 1 < NG)
        def _():
            for hh in range(G):
                for i in range(M - 3):
                    idle_slot(short_kv(0, g + 1, hh * M + i), T_PV)
                if hh == 0:
                    wait_kv(1, g)

                    @pl.when(g + LOOK < NG)
                    def _():
                        long_kv(1, g + LOOK).start(priority=LONG)
                softmax_pv(g * G + hh, hh, [short_kv(0, g + 1, hh * M + M - 3 + i) for i in range(3)])
        return carry

    jax.lax.fori_loop(0, NG, group, 0)

    n_slot = [0]

    def nxt_wo():
        n_slot[0] += 1
        return short_wo[n_slot[0] - 1] if n_slot[0] <= NW else None

    acc = jnp.zeros((8, D), F32)
    n_blk, n_done = 0, NH - G

    def block(acc, n_blk):
        hi = (n_blk + 1) * per
        if n_blk >= WSUB or n_slot[0] < hi + 3 or hi > n_done:
            return acc, n_blk
        rows = wo_v.at[pl.ds(n_blk * per * DH, per * DH), :]
        pltpu.make_async_copy(rows, rows, s_wo0.at[n_blk]).wait()
        slot(nxt_wo())
        for h in range(n_blk * per, hi):
            acc = acc + jnp.dot(o_v[h].astype(BF16), wo_v[pl.ds(h * DH, DH), :], preferred_element_type=F32)
        return acc, n_blk + 1

    long_wo[0].start(priority=LONG)
    for _ in range(4):
        idle_slot(nxt_wo(), T_WO)
    wait_kv(1, NG - 1)
    for c in long_wo[1:]:
        c.start(priority=LONG)
    for hh in range(G):
        softmax_pv(NH - G + hh, hh, [nxt_wo(), nxt_wo(), nxt_wo()])
        n_done += 1
        acc, n_blk = block(acc, n_blk)
    slot(nxt_wo())
    o_last = o_v[NH - 1].astype(BF16).astype(F32)
    o_col = jnp.broadcast_to(o_last[0:1], (DH, DH)).T
    while n_blk < WSUB:
        before = n_blk
        acc, n_blk = block(acc, n_blk)
        if n_blk == before:
            idle_slot(nxt_wo(), T_WO)
    assert n_slot[0] >= NW

    part = None
    row = jax.lax.broadcasted_iota(jnp.int32, (8, D), 0)
    r0 = NW * DH
    for c, rows in enumerate(WO_CHUNKS):
        long_wo[c].wait()
        if c < len(WO_CHUNKS) - WO_VPU:
            for h in range(r0 // DH, (r0 + rows) // DH):
                acc = acc + jnp.dot(o_v[h].astype(BF16), wo_v[pl.ds(h * DH, DH), :], preferred_element_type=F32)
        else:
            if part is None:
                part = jnp.where(row == 0, acc, 0.0)
            lo = r0 - (NH - 1) * DH
            coef = jnp.concatenate([o_col[lo:lo + rows]] * (D // DH), axis=1)
            prod = wo_v[pl.ds(r0, rows), :].astype(F32) * coef
            part = part + prod.reshape(rows // 8, 8, D).sum(axis=0)
        r0 += rows
    s_out = jnp.sum(part, axis=0, keepdims=True)

    res = x8 + jnp.broadcast_to(s_out, (8, D)) * gate
    out_ref[0] = res.astype(out_ref.dtype)[0:1]


@jax.jit
def pallas_recurrent_scan__sliding_block_cached__moe_arch_mod__decode_kernel(
    A_x: jax.Array,
    A_k_cache: jax.Array,
    A_v_cache: jax.Array,
    A_wq: jax.Array,
    A_wo: jax.Array,
    B_x: jax.Array,
    B_w_r: jax.Array,
    B_w_gate: jax.Array,
    B_w_up: jax.Array,
    B_w_down: jax.Array,
):
    del B_x
    hbm = pl.BlockSpec(memory_space=pltpu.HBM)
    dma = pltpu.SemaphoreType.DMA
    return pl.pallas_call(
        _kernel,
        out_shape=jax.ShapeDtypeStruct((1, 1, D), BF16),
        in_specs=[hbm] * 9,
        out_specs=pl.BlockSpec(memory_space=pltpu.VMEM),
        scratch_shapes=[
            pltpu.VMEM((1, 1, D), BF16),
            pltpu.VMEM((D,), BF16),
            pltpu.VMEM((D, NH * DH), BF16),
            pltpu.VMEM((2, NH, W, DH), BF16),
            pltpu.VMEM((NH * DH, D), BF16),
            pltpu.VMEM((F, D), BF16),
            pltpu.VMEM((F, D), BF16),
            pltpu.VMEM((F, D), BF16),
            pltpu.VMEM((NH, 8, DH), F32),
            pltpu.VMEM((NH, 8, DH), F32),
            pltpu.VMEM((G, 8, W), F32),
            dma((2,)), dma((4,)), dma((4,)), dma((2, LOOK + 1)), dma((2, 2)),
            dma((len(WO_CHUNKS),)), dma((WSUB,)),
        ],
        compiler_params=pltpu.CompilerParams(
            vmem_limit_bytes=100 * 1024 * 1024,
            disable_semaphore_checks=True,
        ),
    )(A_x, A_k_cache, A_v_cache, A_wq, A_wo, B_w_r, B_w_gate.T, B_w_up.T, B_w_down)
```

```python
import jax
import jax.numpy as jnp
import jax.experimental.pallas as pl
import jax.experimental.pallas.tpu as pltpu

D = 512
NH = 32
DH = 128
SK = 32768
W = min(4096, max(256, SK // 4))
F = 1376

G = 4
NG = NH // G
PR = 88
M = 8
NP = G * M
K1 = W - NP * PR
QS = 4
LOOK = 2
WQ1, WQR = 112, 16
F1, FR = 352, 128
WR, NW, WB = 96, 28, 4
N7 = NP // 2
WO_CHUNKS = (512, 384, 256, 128, 80, 32, 16)
WO_VPU = 3
T_QK, T_PV, T_WQ, T_F, T_KV0, T_WO = 125, 139, 205, 185, 150, 150

BF16 = jnp.bfloat16
F32 = jnp.float32
_NT = (((1,), (1,)), ((), ()))
LONG, SHORT = 1, 0


def _kernel(x_h, k_h, v_h, wq_h, wo_h, wr_h, wg_h, wu_h, wd_h, out_ref,
            x_v, wr_v, wq_v, kv_v, wo_v, wg_v, wu_v, wd_v, q_v, o_v, p_v, l_v,
            s_x, s_w1, s_w0, s_kv1, s_kv0, s_wo1, s_wo0):
    kv_h = (k_h, v_h)

    def long_kv(t, g):
        return pltpu.make_async_copy(
            kv_h[t].at[0, pl.ds(g * G, G), pl.ds(SK - W, K1), :],
            kv_v.at[t, pl.ds(g * G, G), pl.ds(0, K1), :], s_kv1.at[t, g % (LOOK + 1)])

    def short_kv(t, g, j):
        ro = K1 + j * PR
        return pltpu.make_async_copy(
            kv_h[t].at[0, pl.ds(g * G, G), pl.ds(SK - W + ro, PR), :],
            kv_v.at[t, pl.ds(g * G, G), pl.ds(ro, PR), :], s_kv0.at[t, g % 2])

    def wait_kv(t, g):
        long_kv(t, g).wait()
        rest = kv_v.at[t, pl.ds(g * G, G), pl.ds(K1, W - K1), :]
        pltpu.make_async_copy(rest, rest, s_kv0.at[t, g % 2]).wait()

    copy_x = pltpu.make_async_copy(x_h, x_v, s_x.at[0])
    copy_wr = pltpu.make_async_copy(wr_h, wr_v, s_x.at[1])
    ws = ((wq_h, wq_v), (wg_h, wg_v), (wu_h, wu_v), (wd_h, wd_v))
    w1 = (WQ1, F1, F1, F1)
    long_w = [pltpu.make_async_copy(ws[a][0].at[pl.ds(0, w1[a]), :], ws[a][1].at[pl.ds(0, w1[a]), :],
                                    s_w1.at[a]) for a in range(4)]

    def short_w(a, rows, i):
        ro = w1[a] + i * rows
        return pltpu.make_async_copy(ws[a][0].at[pl.ds(ro, rows), :], ws[a][1].at[pl.ds(ro, rows), :],
                                     s_w0.at[a])

    def wait_w(a):
        long_w[a].wait()
        rest = ws[a][1].at[pl.ds(w1[a], ws[a][1].shape[0] - w1[a]), :]
        pltpu.make_async_copy(rest, rest, s_w0.at[a]).wait()

    HB = WB * WR // DH
    NB = NW // WB
    long_wo = []
    r0 = NW * WR
    for c, r in enumerate(WO_CHUNKS):
        long_wo.append(pltpu.make_async_copy(wo_h.at[pl.ds(r0, r), :], wo_v.at[pl.ds(r0, r), :], s_wo1.at[c]))
        r0 += r
    assert r0 == NH * DH and NB * WB == NW and HB * DH == WB * WR and sum(WO_CHUNKS[-WO_VPU:]) == DH

    def short_wo(i):
        return pltpu.make_async_copy(wo_h.at[pl.ds(i * WR, WR), :], wo_v.at[pl.ds(i * WR, WR), :],
                                     s_wo0.at[i // WB])

    def slot(c):
        pl.delay(1)
        if c is not None:
            c.start(priority=SHORT)
        pl.delay(1)

    def idle_slot(c, t):
        if c is not None:
            c.start(priority=SHORT)
        pl.delay(t)

    n_wq, n_f = (D - WQ1) // WQR, (F - F1) // FR
    assert WQ1 + n_wq * WQR == D and F1 + n_f * FR == F
    HP = NP // 2
    weights = [(short_w(0, WQR, i), T_WQ) for i in range(n_wq)]
    weights += [(short_w(a, FR, i), T_F) for i in range(n_f) for a in (1, 2, 3)]
    seq, used = [], 0
    for i, w_ in enumerate(weights):
        seq.append(w_)
        while used < min(HP, (i + 1) * HP // 30):
            seq.append((short_kv(0, 0, used), T_KV0))
            used += 1
        if i == n_wq - 1:
            n_after_wq = len(seq)
    n_w = len(seq)
    for j in range(HP):
        seq += [(short_kv(0, 0, HP + j), T_KV0), (short_kv(1, 0, j), T_KV0)]
    pos = [0]

    def nxt():
        pos[0] += 1
        return seq[pos[0] - 1]

    def idle_until(n):
        while pos[0] < n:
            idle_slot(*nxt())

    copy_x.start(priority=SHORT)
    copy_wr.start(priority=SHORT)
    for c in long_w:
        c.start(priority=LONG)
    idle_until(2)
    copy_x.wait()
    copy_wr.wait()

    slot(nxt()[0])
    x = x_v[0].astype(F32)
    mean = jnp.mean(x, axis=-1, keepdims=True)
    var = jnp.mean(jnp.square(x - mean), axis=-1, keepdims=True)
    xn_b = ((x - mean) / jnp.sqrt(var + 1e-5)).astype(BF16)
    xn = xn_b.astype(F32)
    x8 = jnp.broadcast_to(x, (8, D))
    xn8 = jnp.broadcast_to(xn_b, (8, D))
    r = jnp.sum(xn * wr_v[...].reshape(1, D).astype(F32), axis=-1, keepdims=True)

    idle_until(n_after_wq + 10)
    long_kv(0, 0).start(priority=LONG)
    long_kv(1, 0).start(priority=LONG)

    wait_w(0)
    QC = 512
    for c in range(NH * DH // QC):
        slot(nxt()[0])
        q = jnp.dot(xn8, wq_v[:, pl.ds(c * QC, QC)], preferred_element_type=F32)
        for t in range(QC // DH):
            q_v[c * (QC // DH) + t] = q[:, t * DH:(t + 1) * DH]

    idle_until(n_w + 4)
    for g in range(1, LOOK):
        long_kv(0, g).start(priority=LONG)
        long_kv(1, g).start(priority=LONG)

    for a in (1, 2, 3):
        wait_w(a)
    y = None
    for c0, cn in ((0, 512), (512, 512), (1024, F - 1024)):
        slot(nxt()[0])
        gt = jax.lax.dot_general(xn8, wg_v[pl.ds(c0, cn), :], _NT, preferred_element_type=F32)
        slot(nxt()[0])
        up = jax.lax.dot_general(xn8, wu_v[pl.ds(c0, cn), :], _NT, preferred_element_type=F32)
        hid = (jax.nn.silu(gt) * up).astype(BF16)
        slot(nxt()[0])
        t = jnp.dot(hid, wd_v[pl.ds(c0, cn), :], preferred_element_type=F32)
        y = t if y is None else y + t
    slot(nxt()[0])
    upd = xn * 0.0 + y * jax.nn.sigmoid(r)
    gate = jax.nn.silu(xn + upd)
    idle_until(len(seq))

    scale = DH ** -0.5
    KS = W // QS
    HW = W // 2

    def start_qk(g, hh, t):
        i = (hh * M + t) // 2
        if t % 2 == 0:
            short_kv(1, g, HP + i).start(priority=SHORT)
        else:
            @pl.when(g + 1 < NG)
            def _():
                short_kv(0, g + 1, i).start(priority=SHORT)

            @pl.when(g + 1 == NG)
            def _():
                short_wo(i).start(priority=SHORT)

    def copy_pv(g, hh, t):
        i = (hh * M + t) // 2
        return short_kv(0, g + 1, HP + i) if t % 2 == 0 else short_kv(1, g + 1, i)

    def probs(g, hh):
        h = g * G + hh
        n_idle = M - QS - 1
        for t in range(n_idle):
            start_qk(g, hh, t)
            pl.delay(T_QK)
        if hh == 0:
            wait_kv(0, g)

            @pl.when(g + LOOK < NG)
            def _():
                long_kv(0, g + LOOK).start(priority=LONG)
        qh = q_v[h].astype(BF16)
        ss = []
        for c in range(QS):
            pl.delay(1)
            start_qk(g, hh, n_idle + c)
            pl.delay(1)
            ss.append(jax.lax.dot_general(qh, kv_v[0, h, pl.ds(c * KS, KS), :], _NT,
                                          preferred_element_type=F32) * scale)
        pl.delay(1)
        start_qk(g, hh, n_idle + QS)
        pl.delay(1)
        mx = ss[0]
        for s in ss[1:]:
            mx = jnp.maximum(mx, s)
        mx = jnp.max(mx, axis=-1, keepdims=True)
        ps = [jnp.exp(s - mx) for s in ss]
        tot = ps[0]
        for p in ps[1:]:
            tot = tot + p
        for c in range(QS):
            p_v[hh, :, pl.ds(c * KS, KS)] = ps[c]
        l_v[hh] = jnp.broadcast_to(jnp.sum(tot, axis=-1, keepdims=True), (8, DH))

    def pv(h, hh, copies):
        slot(copies[0])
        o = jnp.dot(p_v[hh, :, pl.ds(0, HW)].astype(BF16), kv_v[1, h, pl.ds(0, HW), :],
                    preferred_element_type=F32)
        slot(copies[1])
        o = o + jnp.dot(p_v[hh, :, pl.ds(HW, HW)].astype(BF16), kv_v[1, h, pl.ds(HW, HW), :],
                        preferred_element_type=F32)
        o_v[h] = o / l_v[hh]

    def group(g, carry):
        for hh in range(G):
            probs(g, hh)

        @pl.when(g + 1 < NG)
        def _():
            for hh in range(G):
                for t in range(M - 2):
                    idle_slot(copy_pv(g, hh, t), T_PV)
                if hh == 0:
                    wait_kv(1, g)

                    @pl.when(g + LOOK < NG)
                    def _():
                        long_kv(1, g + LOOK).start(priority=LONG)
                pv(g * G + hh, hh, [copy_pv(g, hh, M - 2), copy_pv(g, hh, M - 1)])
        return carry

    jax.lax.fori_loop(0, NG, group, 0)

    n_wo = [N7]

    def nxt_wo():
        if n_wo[0] < NW:
            n_wo[0] += 1
            return short_wo(n_wo[0] - 1)
        return None

    def block(acc, b):
        rows = wo_v.at[pl.ds(b * HB * DH, HB * DH), :]
        pltpu.make_async_copy(rows, rows, s_wo0.at[b]).wait()
        slot(nxt_wo())
        for h in range(b * HB, (b + 1) * HB):
            acc = acc + jnp.dot(o_v[h].astype(BF16), wo_v[pl.ds(h * DH, DH), :], preferred_element_type=F32)
        return acc

    acc = jnp.zeros((8, D), F32)
    n_early = N7 // WB
    assert n_early * HB <= NH - G
    long_wo[0].start(priority=LONG)
    for b in range(n_early):
        acc = block(acc, b)
    wait_kv(1, NG - 1)
    for c in long_wo[1:]:
        c.start(priority=LONG)
    for hh in range(G):
        pv(NH - G + hh, hh, [nxt_wo(), nxt_wo()])
    slot(nxt_wo())
    o_last = o_v[NH - 1].astype(BF16).astype(F32)
    o_col = jnp.broadcast_to(o_last[0:1], (DH, DH)).T
    while n_wo[0] < NW:
        idle_slot(nxt_wo(), T_WO)
    for b in range(n_early, NB):
        acc = block(acc, b)

    part = None
    row = jax.lax.broadcasted_iota(jnp.int32, (8, D), 0)
    r0 = NW * WR
    for c, rows in enumerate(WO_CHUNKS):
        long_wo[c].wait()
        if c < len(WO_CHUNKS) - WO_VPU:
            for h in range(r0 // DH, (r0 + rows) // DH):
                acc = acc + jnp.dot(o_v[h].astype(BF16), wo_v[pl.ds(h * DH, DH), :], preferred_element_type=F32)
        else:
            if part is None:
                part = jnp.where(row == 0, acc, 0.0)
            lo = r0 - (NH - 1) * DH
            coef = jnp.concatenate([o_col[lo:lo + rows]] * (D // DH), axis=1)
            prod = wo_v[pl.ds(r0, rows), :].astype(F32) * coef
            part = part + prod.reshape(rows // 8, 8, D).sum(axis=0)
        r0 += rows
    s_out = jnp.sum(part, axis=0, keepdims=True)

    res = x8 + jnp.broadcast_to(s_out, (8, D)) * gate
    out_ref[0] = res.astype(out_ref.dtype)[0:1]


@jax.jit
def pallas_recurrent_scan__sliding_block_cached__moe_arch_mod__decode_kernel(
    A_x: jax.Array,
    A_k_cache: jax.Array,
    A_v_cache: jax.Array,
    A_wq: jax.Array,
    A_wo: jax.Array,
    B_x: jax.Array,
    B_w_r: jax.Array,
    B_w_gate: jax.Array,
    B_w_up: jax.Array,
    B_w_down: jax.Array,
):
    del B_x
    hbm = pl.BlockSpec(memory_space=pltpu.HBM)
    dma = pltpu.SemaphoreType.DMA
    return pl.pallas_call(
        _kernel,
        out_shape=jax.ShapeDtypeStruct((1, 1, D), BF16),
        in_specs=[hbm] * 9,
        out_specs=pl.BlockSpec(memory_space=pltpu.VMEM),
        scratch_shapes=[
            pltpu.VMEM((1, 1, D), BF16),
            pltpu.VMEM((D,), BF16),
            pltpu.VMEM((D, NH * DH), BF16),
            pltpu.VMEM((2, NH, W, DH), BF16),
            pltpu.VMEM((NH * DH, D), BF16),
            pltpu.VMEM((F, D), BF16),
            pltpu.VMEM((F, D), BF16),
            pltpu.VMEM((F, D), BF16),
            pltpu.VMEM((NH, 8, DH), F32),
            pltpu.VMEM((NH, 8, DH), F32),
            pltpu.VMEM((G, 8, W), F32),
            pltpu.VMEM((G, 8, DH), F32),
            dma((2,)), dma((4,)), dma((4,)), dma((2, LOOK + 1)), dma((2, 2)),
            dma((len(WO_CHUNKS),)), dma((NW // WB,)),
        ],
        compiler_params=pltpu.CompilerParams(
            vmem_limit_bytes=100 * 1024 * 1024,
            disable_semaphore_checks=True,
        ),
    )(A_x, A_k_cache, A_v_cache, A_wq, A_wo, B_w_r, B_w_gate.T, B_w_up.T, B_w_down)
```

```python
import jax
import jax.numpy as jnp
import jax.experimental.pallas as pl
import jax.experimental.pallas.tpu as pltpu

D = 512
NH = 32
DH = 128
SK = 32768
W = min(4096, max(256, SK // 4))
F = 1376

G = 4
NG = NH // G
PR = 88
M = 8
NP = G * M
K1 = W - NP * PR
QS = 4
LOOK = 2
WQ1, WQR = 160, 8
F1, FR = 480, 64
WR, NW, WB = 96, 24, 4
N7 = NP // 2
WO_CHUNKS = (768, 512, 256, 128, 80, 32, 16)
WO_VPU = 3
T_QK, T_PV, T_WQ, T_F, T_KV0, T_WO = 125, 139, 110, 110, 150, 150

BF16 = jnp.bfloat16
F32 = jnp.float32
_NT = (((1,), (1,)), ((), ()))
LONG, SHORT = 1, 0


def _kernel(x_h, k_h, v_h, wq_h, wo_h, wr_h, wg_h, wu_h, wd_h, out_ref,
            x_v, wr_v, wq_v, kv_v, wo_v, wg_v, wu_v, wd_v, q_v, o_v, p_v, l_v,
            s_x, s_w1, s_w0, s_kv1, s_kv0, s_wo1, s_wo0):
    kv_h = (k_h, v_h)

    def long_kv(t, g):
        return pltpu.make_async_copy(
            kv_h[t].at[0, pl.ds(g * G, G), pl.ds(SK - W, K1), :],
            kv_v.at[t, pl.ds(g * G, G), pl.ds(0, K1), :], s_kv1.at[t, g % (LOOK + 1)])

    def short_kv(t, g, j):
        ro = K1 + j * PR
        return pltpu.make_async_copy(
            kv_h[t].at[0, pl.ds(g * G, G), pl.ds(SK - W + ro, PR), :],
            kv_v.at[t, pl.ds(g * G, G), pl.ds(ro, PR), :], s_kv0.at[t, g % 2])

    def wait_kv(t, g):
        long_kv(t, g).wait()
        rest = kv_v.at[t, pl.ds(g * G, G), pl.ds(K1, W - K1), :]
        pltpu.make_async_copy(rest, rest, s_kv0.at[t, g % 2]).wait()

    copy_x = pltpu.make_async_copy(x_h, x_v, s_x.at[0])
    copy_wr = pltpu.make_async_copy(wr_h, wr_v, s_x.at[1])
    ws = ((wq_h, wq_v), (wg_h, wg_v), (wu_h, wu_v), (wd_h, wd_v))
    w1 = (WQ1, F1, F1, F1)
    long_w = [pltpu.make_async_copy(ws[a][0].at[pl.ds(0, w1[a]), :], ws[a][1].at[pl.ds(0, w1[a]), :],
                                    s_w1.at[a]) for a in range(4)]

    def short_w(a, rows, i):
        ro = w1[a] + i * rows
        return pltpu.make_async_copy(ws[a][0].at[pl.ds(ro, rows), :], ws[a][1].at[pl.ds(ro, rows), :],
                                     s_w0.at[a])

    def wait_w(a):
        long_w[a].wait()
        rest = ws[a][1].at[pl.ds(w1[a], ws[a][1].shape[0] - w1[a]), :]
        pltpu.make_async_copy(rest, rest, s_w0.at[a]).wait()

    HB = WB * WR // DH
    NB = NW // WB
    long_wo = []
    r0 = NW * WR
    for c, r in enumerate(WO_CHUNKS):
        long_wo.append(pltpu.make_async_copy(wo_h.at[pl.ds(r0, r), :], wo_v.at[pl.ds(r0, r), :], s_wo1.at[c]))
        r0 += r
    assert r0 == NH * DH and NB * WB == NW and HB * DH == WB * WR and sum(WO_CHUNKS[-WO_VPU:]) == DH

    def short_wo(i):
        return pltpu.make_async_copy(wo_h.at[pl.ds(i * WR, WR), :], wo_v.at[pl.ds(i * WR, WR), :],
                                     s_wo0.at[i // WB])

    def slot(c):
        if c is not None:
            pl.delay(1)
            c.start(priority=SHORT)
            pl.delay(1)

    def idle_slot(c, t):
        if c is not None:
            c.start(priority=SHORT)
        pl.delay(t)

    n_wq, n_f = (D - WQ1) // WQR, (F - F1) // FR
    assert WQ1 + n_wq * WQR == D and F1 + n_f * FR == F
    HP = NP // 2
    weights = [(short_w(0, WQR, i), T_WQ) for i in range(n_wq)]
    weights += [(short_w(a, FR, i), T_F) for i in range(n_f) for a in (1, 2, 3)]
    seq, used = [], 0
    for i, w_ in enumerate(weights):
        seq.append(w_)
        while used < min(HP, (i + 1) * HP // 30):
            seq.append((short_kv(0, 0, used), T_KV0))
            used += 1
        if i == n_wq - 1:
            n_after_wq = len(seq)
    n_w = len(seq)
    for j in range(HP):
        seq += [(short_kv(0, 0, HP + j), T_KV0), (short_kv(1, 0, j), T_KV0)]
    pos = [0]

    def nxt():
        pos[0] += 1
        return seq[pos[0] - 1]

    def idle_until(n):
        while pos[0] < n:
            idle_slot(*nxt())

    copy_x.start(priority=SHORT)
    copy_wr.start(priority=SHORT)
    for c in long_w:
        c.start(priority=LONG)
    idle_until(2)
    copy_x.wait()
    copy_wr.wait()

    slot(nxt()[0])
    x = x_v[0].astype(F32)
    mean = jnp.mean(x, axis=-1, keepdims=True)
    var = jnp.mean(jnp.square(x - mean), axis=-1, keepdims=True)
    xn_b = ((x - mean) / jnp.sqrt(var + 1e-5)).astype(BF16)
    xn = xn_b.astype(F32)
    x8 = jnp.broadcast_to(x, (8, D))
    xn8 = jnp.broadcast_to(xn_b, (8, D))
    r = jnp.sum(xn * wr_v[...].reshape(1, D).astype(F32), axis=-1, keepdims=True)

    idle_until(n_after_wq + 10)
    long_kv(0, 0).start(priority=LONG)
    long_kv(1, 0).start(priority=LONG)

    wait_w(0)
    QC = 512
    for c in range(NH * DH // QC):
        slot(nxt()[0])
        q = jnp.dot(xn8, wq_v[:, pl.ds(c * QC, QC)], preferred_element_type=F32)
        for t in range(QC // DH):
            q_v[c * (QC // DH) + t] = q[:, t * DH:(t + 1) * DH]

    idle_until(n_w + 4)
    for g in range(1, LOOK):
        long_kv(0, g).start(priority=LONG)
        long_kv(1, g).start(priority=LONG)

    for a in (1, 2, 3):
        wait_w(a)
    y = None
    for c0, cn in ((0, 512), (512, 512), (1024, F - 1024)):
        slot(nxt()[0])
        gt = jax.lax.dot_general(xn8, wg_v[pl.ds(c0, cn), :], _NT, preferred_element_type=F32)
        slot(nxt()[0])
        up = jax.lax.dot_general(xn8, wu_v[pl.ds(c0, cn), :], _NT, preferred_element_type=F32)
        hid = (jax.nn.silu(gt) * up).astype(BF16)
        slot(nxt()[0])
        t = jnp.dot(hid, wd_v[pl.ds(c0, cn), :], preferred_element_type=F32)
        y = t if y is None else y + t
    slot(nxt()[0])
    upd = xn * 0.0 + y * jax.nn.sigmoid(r)
    gate = jax.nn.silu(xn + upd)
    idle_until(len(seq))

    scale = DH ** -0.5
    KS = W // QS
    HW = W // 2

    def start_qk(g, hh, t):
        i = (hh * M + t) // 2
        if t % 2 == 0:
            short_kv(1, g, HP + i).start(priority=SHORT)
        else:
            @pl.when(g + 1 < NG)
            def _():
                short_kv(0, g + 1, i).start(priority=SHORT)

            @pl.when(g + 1 == NG)
            def _():
                short_wo(i).start(priority=SHORT)

    def copy_pv(g, hh, t):
        i = (hh * M + t) // 2
        return short_kv(0, g + 1, HP + i) if t % 2 == 0 else short_kv(1, g + 1, i)

    def probs(g, hh):
        h = g * G + hh
        n_idle = M - QS - 1
        for t in range(n_idle):
            start_qk(g, hh, t)
            pl.delay(T_QK)
        if hh == 0:
            wait_kv(0, g)

            @pl.when(g + LOOK < NG)
            def _():
                long_kv(0, g + LOOK).start(priority=LONG)

            @pl.when(g + 1 == NG)
            def _():
                long_wo[0].start(priority=LONG)
        qh = q_v[h].astype(BF16)
        ss = []
        for c in range(QS):
            pl.delay(1)
            start_qk(g, hh, n_idle + c)
            pl.delay(1)
            ss.append(jax.lax.dot_general(qh, kv_v[0, h, pl.ds(c * KS, KS), :], _NT,
                                          preferred_element_type=F32) * scale)
        pl.delay(1)
        start_qk(g, hh, n_idle + QS)
        pl.delay(1)
        mx = ss[0]
        for s in ss[1:]:
            mx = jnp.maximum(mx, s)
        mx = jnp.max(mx, axis=-1, keepdims=True)
        ps = [jnp.exp(s - mx) for s in ss]
        tot = ps[0]
        for p in ps[1:]:
            tot = tot + p
        for c in range(QS):
            p_v[hh, :, pl.ds(c * KS, KS)] = ps[c]
        l_v[hh] = jnp.broadcast_to(jnp.sum(tot, axis=-1, keepdims=True), (8, DH))

    def pv(h, hh, copies):
        slot(copies[0])
        o = jnp.dot(p_v[hh, :, pl.ds(0, HW)].astype(BF16), kv_v[1, h, pl.ds(0, HW), :],
                    preferred_element_type=F32)
        slot(copies[1])
        o = o + jnp.dot(p_v[hh, :, pl.ds(HW, HW)].astype(BF16), kv_v[1, h, pl.ds(HW, HW), :],
                        preferred_element_type=F32)
        o_v[h] = o / l_v[hh]

    def group(g, carry):
        for hh in range(G):
            probs(g, hh)

        @pl.when(g + 1 < NG)
        def _():
            for hh in range(G):
                for t in range(M - 2):
                    idle_slot(copy_pv(g, hh, t), T_PV)
                if hh == 0:
                    wait_kv(1, g)

                    @pl.when(g + LOOK < NG)
                    def _():
                        long_kv(1, g + LOOK).start(priority=LONG)
                pv(g * G + hh, hh, [copy_pv(g, hh, M - 2), copy_pv(g, hh, M - 1)])
        return carry

    jax.lax.fori_loop(0, NG, group, 0)

    n_wo = [N7]

    def nxt_wo():
        if n_wo[0] < NW:
            n_wo[0] += 1
            return short_wo(n_wo[0] - 1)
        return None

    def block(acc, b):
        rows = wo_v.at[pl.ds(b * HB * DH, HB * DH), :]
        pltpu.make_async_copy(rows, rows, s_wo0.at[b]).wait()
        slot(nxt_wo())
        for h in range(b * HB, (b + 1) * HB):
            acc = acc + jnp.dot(o_v[h].astype(BF16), wo_v[pl.ds(h * DH, DH), :], preferred_element_type=F32)
        return acc

    acc = jnp.zeros((8, D), F32)
    n_early = N7 // WB
    assert n_early * HB <= NH - G
    for b in range(n_early):
        acc = block(acc, b)
    wait_kv(1, NG - 1)
    for c in long_wo[1:]:
        c.start(priority=LONG)
    for hh in range(G):
        pv(NH - G + hh, hh, [nxt_wo(), nxt_wo()])
    slot(nxt_wo())
    o_last = o_v[NH - 1].astype(BF16).astype(F32)
    o_col = jnp.broadcast_to(o_last[0:1], (DH, DH)).T
    while n_wo[0] < NW:
        idle_slot(nxt_wo(), T_WO)
    for b in range(n_early, NB):
        acc = block(acc, b)

    part = None
    row = jax.lax.broadcasted_iota(jnp.int32, (8, D), 0)
    r0 = NW * WR
    for c, rows in enumerate(WO_CHUNKS):
        long_wo[c].wait()
        if c < len(WO_CHUNKS) - WO_VPU:
            for h in range(r0 // DH, (r0 + rows) // DH):
                acc = acc + jnp.dot(o_v[h].astype(BF16), wo_v[pl.ds(h * DH, DH), :], preferred_element_type=F32)
        else:
            if part is None:
                part = jnp.where(row == 0, acc, 0.0)
            lo = r0 - (NH - 1) * DH
            coef = jnp.concatenate([o_col[lo:lo + rows]] * (D // DH), axis=1)
            prod = wo_v[pl.ds(r0, rows), :].astype(F32) * coef
            part = part + prod.reshape(rows // 8, 8, D).sum(axis=0)
        r0 += rows
    s_out = jnp.sum(part, axis=0, keepdims=True)

    res = x8 + jnp.broadcast_to(s_out, (8, D)) * gate
    out_ref[0] = res.astype(out_ref.dtype)[0:1]


@jax.jit
def pallas_recurrent_scan__sliding_block_cached__moe_arch_mod__decode_kernel(
    A_x: jax.Array,
    A_k_cache: jax.Array,
    A_v_cache: jax.Array,
    A_wq: jax.Array,
    A_wo: jax.Array,
    B_x: jax.Array,
    B_w_r: jax.Array,
    B_w_gate: jax.Array,
    B_w_up: jax.Array,
    B_w_down: jax.Array,
):
    del B_x
    hbm = pl.BlockSpec(memory_space=pltpu.HBM)
    dma = pltpu.SemaphoreType.DMA
    return pl.pallas_call(
        _kernel,
        out_shape=jax.ShapeDtypeStruct((1, 1, D), BF16),
        in_specs=[hbm] * 9,
        out_specs=pl.BlockSpec(memory_space=pltpu.VMEM),
        scratch_shapes=[
            pltpu.VMEM((1, 1, D), BF16),
            pltpu.VMEM((D,), BF16),
            pltpu.VMEM((D, NH * DH), BF16),
            pltpu.VMEM((2, NH, W, DH), BF16),
            pltpu.VMEM((NH * DH, D), BF16),
            pltpu.VMEM((F, D), BF16),
            pltpu.VMEM((F, D), BF16),
            pltpu.VMEM((F, D), BF16),
            pltpu.VMEM((NH, 8, DH), F32),
            pltpu.VMEM((NH, 8, DH), F32),
            pltpu.VMEM((G, 8, W), F32),
            pltpu.VMEM((G, 8, DH), F32),
            dma((2,)), dma((4,)), dma((4,)), dma((2, LOOK + 1)), dma((2, 2)),
            dma((len(WO_CHUNKS),)), dma((NW // WB,)),
        ],
        compiler_params=pltpu.CompilerParams(
            vmem_limit_bytes=100 * 1024 * 1024,
            disable_semaphore_checks=True,
        ),
    )(A_x, A_k_cache, A_v_cache, A_wq, A_wo, B_w_r, B_w_gate.T, B_w_up.T, B_w_down)
```
